```python
import os as _os
_os.environ.setdefault("JAX_PLATFORMS", "cpu")
import jax
import jax.numpy as jnp

def _softmax(x, axis=-1):
    return jax.nn.softmax(x, axis=axis)
def _gelu(x):
    return jax.nn.gelu(x, approximate=True)
def _silu(x):
    return jax.nn.silu(x)
def _sigmoid(x):
    return jax.nn.sigmoid(x)
def _layernorm(x, axis=-1, eps=1e-5):
    m = jnp.mean(x, axis=axis, keepdims=True)
    v = jnp.var(x, axis=axis, keepdims=True)
    return (x - m) / jnp.sqrt(v + eps)
def _scatter_add(tgt, idx, src, axis=0):
    return tgt.at[idx].add(src)
def _segment_sum(src, seg, n):
    return jax.ops.segment_sum(src, seg, n)
class _Rng:
    def __init__(self, key):
        self._k = key
    def _next(self):
        self._k, sub = jax.random.split(self._k)
        return sub
    def normal(self, shape):
        return jax.random.normal(self._next(), shape, dtype=jnp.bfloat16)
    def randint(self, lo, hi, shape):
        return jax.random.randint(self._next(), shape, lo, hi, dtype=jnp.int32)
    def uniform(self, shape, lo=0.0, hi=1.0):
        return jax.random.uniform(self._next(), shape, jnp.bfloat16, lo, hi)
    def permutation(self, n):
        return jax.random.permutation(self._next(), n)


kernel_name = 'concat_heads__mha_block__ssm_conv_s4__prompt'

def setup_inputs():
    _rng = _Rng(jax.random.key(int.from_bytes(__import__("os").urandom(4), "little")))
    _w = (lambda a: (lambda t: t.astype(jnp.bfloat16) if jnp.issubdtype(t.dtype, jnp.floating) else t)(jnp.asarray(a)))
    def _A_setup():
        B, S, D, H = 1, 2048, 448, 16
        return {
            "x": _w((lambda *s: _rng.normal(s) * 0.2)(B, S, D)),
            "wqkv": _w((lambda *s: _rng.normal(s) * 0.2)(D, 3 * D)),
            "wo": _w((lambda *s: _rng.normal(s) * 0.05)(D, D)),
        }
    _A_in = _A_setup()

    def _B_setup():
        B, L, D, N = 1, 2048, 448, 256
        A_re = -jnp.exp((lambda *s: _rng.normal(s) * 0.2)(D, N))
        A_im = jnp.pi * (lambda *s: _rng.normal(s) * 0.2)(D, N)
        B_re = (lambda *s: _rng.normal(s) * 0.2)(D, N)
        B_im = (lambda *s: _rng.normal(s) * 0.2)(D, N)
        C_re = (lambda *s: _rng.normal(s) * 0.2)(D, N)
        C_im = (lambda *s: _rng.normal(s) * 0.2)(D, N)
        log_dt = (lambda *s: _rng.normal(s) * 0.2)(D) * 0.5 - 4.0
        Dskip = (lambda *s: _rng.normal(s) * 0.05)(D)
        return {
            "u": _w((lambda *s: _rng.normal(s) * 0.05)(B, L, D)),
            "A_re": _w(A_re),
            "A_im": _w(A_im),
            "B_re": _w(B_re),
            "B_im": _w(B_im),
            "C_re": _w(C_re),
            "C_im": _w(C_im),
            "log_dt": _w(log_dt),
            "Dskip": _w(Dskip),
        }
    _B_in = _B_setup()

    return {
        "A_x": _A_in["x"],
        "A_wqkv": _A_in["wqkv"],
        "A_wo": _A_in["wo"],
        "B_u": _B_in["u"],
        "B_A_re": _B_in["A_re"],
        "B_A_im": _B_in["A_im"],
        "B_B_re": _B_in["B_re"],
        "B_B_im": _B_in["B_im"],
        "B_C_re": _B_in["C_re"],
        "B_C_im": _B_in["C_im"],
        "B_log_dt": _B_in["log_dt"],
        "B_Dskip": _B_in["Dskip"],
    }

def reference(A_x, A_wqkv, A_wo, B_u, B_A_re, B_A_im, B_B_re, B_B_im, B_C_re, B_C_im, B_log_dt, B_Dskip):
    def _A_ref(x, wqkv, wo):
        B, S, D = x.shape
        H = 16
        Dh = D // H
        qkv = (lambda x, *d: x.transpose(*d))((x @ wqkv).reshape(B, S, 3, H, Dh), 2, 0, 3, 1, 4)
        q, k, v = qkv[0], qkv[1], qkv[2]
        scores = jnp.einsum("bhqd,bhkd->bhqk", q, k) * (Dh ** -0.5)
        p = _softmax(scores, axis=-1)
        o = jnp.einsum("bhqk,bhkd->bhqd", p, v)
        return (lambda x, *d: x.transpose(*d))(o, 0, 2, 1, 3).reshape(B, S, D) @ wo

    def _B_ref(u, A_re, A_im, B_re, B_im, C_re, C_im, log_dt, Dskip):
        Bsz, L, D = u.shape
        dt = jnp.exp(log_dt)[:, None]
        A = A_re + 1j * A_im
        Bc = B_re + 1j * B_im
        Cc = C_re + 1j * C_im
        logdA = dt * A
        dB = dt * Bc
        l = (lambda x, dt: x.astype(dt))(jnp.arange(L), A_re.dtype)
        P = jnp.exp(logdA[:, :, None] * l[None, None, :])
        K = jnp.einsum("dn,dnl,dn->dl", Cc, P, dB).real
        L2 = 2 * L
        Kp = jnp.pad(K, ((0, 0), (0, L)))
        up = (lambda x, *d: x.transpose(*d))(u, 0, 2, 1)
        up = jnp.pad(up, ((0, 0), (0, 0), (0, L)))
        Kf = (lambda x, axes=(-2,-1): jnp.fft.rfft2(x.astype(jnp.float32), axes=axes))(Kp[:, None, :], axes=(-2, -1))
        Uf = (lambda x, axes=(-2,-1): jnp.fft.rfft2(x.astype(jnp.float32), axes=axes))(up[:, :, None, :], axes=(-2, -1))
        Yf = Uf * Kf[None, :, :, :]
        y = (lambda x, s, axes=(-2,-1): jnp.fft.irfft2(x, s=s, axes=axes).astype(jnp.bfloat16))(Yf, (1, L2), axes=(-2, -1))[:, :, 0, :L]
        y = (lambda x, *d: x.transpose(*d))(y, 0, 2, 1) + u * Dskip[None, None, :]
        return y

    a = _A_ref(A_x, A_wqkv, A_wo)
    b = _B_ref(B_u, B_A_re, B_A_im, B_B_re, B_B_im, B_C_re, B_C_im, B_log_dt, B_Dskip)
    return jnp.concatenate([a, b], axis=-1)
```

```python
import functools

import numpy as np
import jax
import jax.numpy as jnp
from jax import lax
import jax.experimental.pallas as pl
import jax.experimental.pallas.tpu as pltpu

S = 2048
D = 448
H = 16
DH = 28
HP = 32
DP = H * HP
NS = 256
L2 = 4096
R = 64
TQ = 256
NB = 32
NV = 648


def _dft_constants():
    a = np.arange(32)
    k1 = np.arange(R)
    b = np.arange(R)
    k2 = np.arange(R)
    th = -2.0 * np.pi * np.outer(k1, a) / R
    f1 = np.concatenate([np.cos(th), np.sin(th)], axis=0)
    kk = k1[:, None, None] + R * k2[None, :, None]
    th = -2.0 * np.pi * (kk * b[None, None, :] % L2) / L2
    wr, wi = np.cos(th), np.sin(th)
    g = np.concatenate(
        [np.concatenate([wr, -wi], axis=2), np.concatenate([wi, wr], axis=2)], axis=1)
    wr, wi = np.transpose(wr, (0, 2, 1)), -np.transpose(wi, (0, 2, 1))
    h = np.concatenate(
        [np.concatenate([wr, -wi], axis=2), np.concatenate([wi, wr], axis=2)], axis=1)
    th = 2.0 * np.pi * np.outer(a, k1) / R
    f2 = np.concatenate([np.cos(th), -np.sin(th)], axis=1) / L2
    bf = jnp.bfloat16
    return (jnp.asarray(f1, bf), jnp.asarray(g, bf), jnp.asarray(h, bf), jnp.asarray(f2, bf))


def _cexp(re, im):
    e = jnp.exp(re)
    return e * jnp.cos(im), e * jnp.sin(im)


def _kernel(x_ref, w_ref, wo_ref, u_ref, are_ref, aim_ref, bre_ref, bim_ref,
            cre_ref, cim_ref, ldt_ref, dsk_ref, f1_ref, g_ref, h_ref, f2_ref,
            out_ref,
            q_s, kt_s, vm_s, lor_s, loi_s, hir_s, hii_s, kacc_s, ktime_s,
            a1u_s, a1k_s, uf_s, yh_s):
    f32, bf16 = jnp.float32, jnp.bfloat16

    lane = lax.broadcasted_iota(jnp.int32, (TQ, 128), 1)

    def proj(i, c):
        r0 = pl.multiple_of(i * TQ, TQ)
        xb = x_ref[pl.ds(r0, TQ), :]
        qkv = jnp.dot(xb, w_ref[...], preferred_element_type=f32)
        q_s[pl.ds(r0, TQ), :] = (qkv[:, :DP] * (DH ** -0.5)).astype(bf16)
        kt_s[:, pl.ds(r0, TQ)] = qkv[:, DP:2 * DP].T.astype(bf16)
        for g in range(4):
            vg = qkv[:, 2 * DP + 128 * g: 2 * DP + 128 * (g + 1)]
            for hh in range(4):
                lo = HP * hh
                vmask = jnp.where((lane >= lo) & (lane < lo + DH), vg, 0.0)
                vmask = jnp.where(lane == lo + DH, 1.0, vmask)
                vm_s[4 * g + hh, pl.ds(r0, TQ), :] = vmask.astype(bf16)
        return c

    lax.fori_loop(0, S // TQ, proj, 0)

    def attn(i, c):
        r0 = pl.multiple_of(i * TQ, TQ)
        outs = []
        for g in range(4):
            qg = q_s[pl.ds(r0, TQ), 128 * g:128 * (g + 1)]
            ktg = kt_s[128 * g:128 * (g + 1), :]
            og = jnp.zeros((TQ, 128), f32)
            for hh in range(4):
                lo = HP * hh
                qm = jnp.where((lane >= lo) & (lane < lo + DH), qg, jnp.zeros_like(qg))
                s = jnp.dot(qm, ktg, preferred_element_type=f32)
                m = jnp.max(s, axis=-1, keepdims=True)
                p = jnp.exp(s - m).astype(bf16)
                oh = jnp.dot(p, vm_s[4 * g + hh], preferred_element_type=f32)
                l = oh[:, lo + DH:lo + DH + 1]
                og = og + oh * (1.0 / l)
            outs.append(og.astype(bf16))
        o = jnp.concatenate(outs, axis=1)
        res = jnp.dot(o, wo_ref[...], preferred_element_type=f32)
        out_ref[pl.ds(r0, TQ), 0:D] = res.astype(out_ref.dtype)
        return c

    lax.fori_loop(0, S // TQ, attn, 0)

    dt = jnp.exp(ldt_ref[...].astype(f32)).astype(bf16).astype(f32)
    kacc_s[...] = jnp.zeros_like(kacc_s)

    def kgen(nb, c):
        n0 = pl.multiple_of(nb * NB, NB)
        rows = pl.ds(n0, NB)
        ar = dt * are_ref[rows, :].astype(f32)
        ai = dt * aim_ref[rows, :].astype(f32)
        dbr = dt * bre_ref[rows, :].astype(f32)
        dbi = dt * bim_ref[rows, :].astype(f32)
        cr = cre_ref[rows, :].astype(f32)
        ci = cim_ref[rows, :].astype(f32)
        cbr = cr * dbr - ci * dbi
        cbi = cr * dbi + ci * dbr

        def lo_body(j, c2):
            seg = j // 16
            e = (lax.shift_left(1, seg) * (j % 16)).astype(f32)
            zr, zi = _cexp(ar * e, ai * e)
            lor_s[j] = zr
            loi_s[j] = zi
            return c2
        lax.fori_loop(0, 64, lo_body, 0)

        def hi_body(j, c2):
            seg = jnp.where(j < 16, 0, (j - 16) // 8 + 1)
            hidx = jnp.where(j < 16, j, (j - 16) % 8)
            base = jnp.where(j < 16, 0, lax.shift_left(128, seg))
            e = (base + lax.shift_left(16, seg) * hidx).astype(f32)
            zr, zi = _cexp(ar * e, ai * e)
            hir_s[j] = cbr * zr - cbi * zi
            hii_s[j] = cbr * zi + cbi * zr
            return c2
        lax.fori_loop(0, 41, hi_body, 0)

        def pair_body(j, c2):
            seg = jnp.where(j < 16, 0, (j - 16) // 8 + 1)
            hr = hir_s[j]
            hi = hii_s[j]
            for cc in range(16):
                t = lor_s[16 * seg + cc] * hr - loi_s[16 * seg + cc] * hi
                v = 16 * j + cc
                kacc_s[v] += t.reshape(NB // 8, 8, D).sum(axis=0)
            return c2
        lax.fori_loop(0, 40, pair_body, 0)
        kacc_s[640] += hir_s[40].reshape(NB // 8, 8, D).sum(axis=0)
        return c

    lax.fori_loop(0, NS // NB, kgen, 0)

    def chunks(val):
        rows = val.shape[0]
        return [val[:, 0:128], val[:, 128:256], val[:, 256:384],
                jnp.concatenate([val[:, 384:448], jnp.zeros((rows, 64), val.dtype)], axis=1)]

    def red(i, c):
        r0 = pl.multiple_of(i * 8, 8)
        kv = jnp.sum(kacc_s[pl.ds(r0, 8)], axis=1)
        for ch, part in enumerate(chunks(kv)):
            ktime_s[ch, pl.ds(r0, 8), :] = part
        return c
    lax.fori_loop(0, NV // 8, red, 0)
    KT0 = 1024
    for ch in range(4):
        ktime_s[ch, pl.ds(KT0, 256), :] = ktime_s[ch, pl.ds(0, 256), :]
        for j, off in enumerate((0, 0, 1, 2)):
            ktime_s[ch, pl.ds(KT0 + 256 + j, 64, stride=4), :] = (
                ktime_s[ch, pl.ds(256 + off, 64, stride=2), :])
        for j, off in enumerate((0, 0, 0, 1, 1, 1, 2, 2)):
            ktime_s[ch, pl.ds(KT0 + 512 + j, 64, stride=8), :] = (
                ktime_s[ch, pl.ds(384 + off, 64, stride=2), :])
        for j, off in enumerate((0,) * 5 + (1,) * 7 + (2,) * 4):
            ktime_s[ch, pl.ds(KT0 + 1024 + j, 64, stride=16), :] = (
                ktime_s[ch, pl.ds(512 + off, 64, stride=2), :])

    def ucp(i, c):
        r0 = pl.multiple_of(i * TQ, TQ)
        for ch, part in enumerate(chunks(u_ref[pl.ds(r0, TQ), :].astype(f32))):
            uf_s[ch, pl.ds(r0, TQ), :] = part
        return c
    lax.fori_loop(0, S // TQ, ucp, 0)

    def st1(b, c):
        for ch in range(4):
            xu = uf_s[ch, pl.ds(b, 32, stride=R), :].astype(bf16)
            xk = ktime_s[ch, pl.ds(KT0 + b, 32, stride=R), :].astype(bf16)
            r0 = pl.multiple_of(b * 128, 128)
            a1u_s[ch, pl.ds(r0, 128), :] = jnp.dot(f1_ref[...], xu, preferred_element_type=f32)
            a1k_s[ch, pl.ds(r0, 128), :] = jnp.dot(f1_ref[...], xk, preferred_element_type=f32)
        return c
    lax.fori_loop(0, R, st1, 0)

    def st2(k1, c):
        gk = g_ref[k1]
        hk = h_ref[k1]
        for ch in range(4):
            au = jnp.concatenate([a1u_s[ch, pl.ds(k1, R, stride=128), :],
                                  a1u_s[ch, pl.ds(R + k1, R, stride=128), :]], axis=0).astype(bf16)
            ak = jnp.concatenate([a1k_s[ch, pl.ds(k1, R, stride=128), :],
                                  a1k_s[ch, pl.ds(R + k1, R, stride=128), :]], axis=0).astype(bf16)
            uh = jnp.dot(gk, au, preferred_element_type=f32)
            kh = jnp.dot(gk, ak, preferred_element_type=f32)
            ur, ui = uh[:R], uh[R:]
            kr, ki = kh[:R], kh[R:]
            yh = jnp.concatenate([ur * kr - ui * ki, ur * ki + ui * kr], axis=0).astype(bf16)
            r0 = pl.multiple_of(k1 * 128, 128)
            yh_s[ch, pl.ds(r0, 128), :] = jnp.dot(hk, yh, preferred_element_type=f32)
        return c
    lax.fori_loop(0, R, st2, 0)

    dsk = chunks(dsk_ref[...].astype(f32))

    def st3(b, c):
        for ch in range(4):
            bb = jnp.concatenate([yh_s[ch, pl.ds(b, R, stride=128), :],
                                  yh_s[ch, pl.ds(R + b, R, stride=128), :]], axis=0).astype(bf16)
            y = jnp.dot(f2_ref[...], bb, preferred_element_type=f32)
            ub = uf_s[ch, pl.ds(b, 32, stride=R), :]
            y = y.astype(bf16).astype(f32) + (ub * dsk[ch]).astype(bf16).astype(f32)
            ktime_s[ch, pl.ds(b, 32, stride=R), :] = y
        return c
    lax.fori_loop(0, R, st3, 0)

    def wout(i, c):
        r0 = pl.multiple_of(i * TQ, TQ)
        y = jnp.concatenate([ktime_s[ch, pl.ds(r0, TQ), :] for ch in range(3)]
                            + [ktime_s[3, pl.ds(r0, TQ), 0:64]], axis=1)
        out_ref[pl.ds(r0, TQ), D:2 * D] = y.astype(out_ref.dtype)
        return c
    lax.fori_loop(0, S // TQ, wout, 0)


@jax.jit
def pallas_concat_heads__mha_block__ssm_conv_s4__prompt_kernel(
    A_x: jax.Array,
    A_wqkv: jax.Array,
    A_wo: jax.Array,
    B_u: jax.Array,
    B_A_re: jax.Array,
    B_A_im: jax.Array,
    B_B_re: jax.Array,
    B_B_im: jax.Array,
    B_C_re: jax.Array,
    B_C_im: jax.Array,
    B_log_dt: jax.Array,
    B_Dskip: jax.Array,
):
    bf16, f32 = jnp.bfloat16, jnp.float32
    x = A_x.reshape(S, D)
    w = jnp.pad(A_wqkv.reshape(D, 3 * H, DH), ((0, 0), (0, 0), (0, HP - DH))).reshape(D, 3 * DP)
    wo = jnp.pad(A_wo.reshape(H, DH, D), ((0, 0), (0, HP - DH), (0, 0))).reshape(DP, D)
    u = B_u.reshape(S, D)
    ssm = [a.T for a in (B_A_re, B_A_im, B_B_re, B_B_im, B_C_re, B_C_im)]
    ldt = B_log_dt.reshape(1, D)
    dsk = B_Dskip.reshape(1, D)
    f1, g, h, f2 = _dft_constants()

    scratch = [
        pltpu.VMEM((S, DP), bf16),
        pltpu.VMEM((DP, S), bf16),
        pltpu.VMEM((H, S, 128), bf16),
        pltpu.VMEM((64, NB, D), f32),
        pltpu.VMEM((64, NB, D), f32),
        pltpu.VMEM((41, NB, D), f32),
        pltpu.VMEM((41, NB, D), f32),
        pltpu.VMEM((NV, 8, D), f32),
        pltpu.VMEM((4, 3072, 128), f32),
        pltpu.VMEM((4, R * 128, 128), f32),
        pltpu.VMEM((4, R * 128, 128), f32),
        pltpu.VMEM((4, S, 128), f32),
        pltpu.VMEM((4, R * 128, 128), f32),
    ]
    out = pl.pallas_call(
        _kernel,
        out_shape=jax.ShapeDtypeStruct((S, 2 * D), bf16),
        scratch_shapes=scratch,
        compiler_params=pltpu.CompilerParams(vmem_limit_bytes=120 * 1024 * 1024),
    )(x, w, wo, u, *ssm, ldt, dsk, f1, g, h, f2)
    return out.reshape(1, S, 2 * D)
```

```python
import functools

import numpy as np
import jax
import jax.numpy as jnp
from jax import lax
import jax.experimental.pallas as pl
import jax.experimental.pallas.tpu as pltpu

S = 2048
D = 448
H = 16
DH = 28
HP = 32
DP = H * HP
NS = 256
BL = 128
FL = 256
NBLK = S // BL
NVP = 768
TQ = 256
NB = 16
D2 = 2 * D
NV = 648


def _bf16_round_positions():
    t = np.arange(S)
    idx = np.empty(S, np.int64)
    for i, tt in enumerate(t):
        if tt < 256:
            idx[i] = tt
            continue
        seg = int(np.floor(np.log2(tt))) - 7
        step = 1 << seg
        base = 128 << seg
        q, r = divmod(tt - base, step)
        if 2 * r > step or (2 * r == step and q % 2 == 1):
            q += 1
        idx[i] = 128 + 128 * seg + q
    return idx


def _window_tile(m):
    return (0, 1, 2, 2, 3, 3, 3, 3, 4, 4, 4, 4, 4, 4, 4, 4)[m]


def _dft_constants():
    j = np.arange(BL)[:, None]
    k = np.arange(BL)[None, :]
    fwd = np.concatenate([np.cos(2 * np.pi * j * k / FL), -np.sin(2 * np.pi * j * k / FL)], axis=1)
    fwd[:, BL] = np.cos(np.pi * j[:, 0])
    jj = np.arange(FL)[None, :]
    kk = np.arange(BL)[:, None]
    inv = np.concatenate([2 * np.cos(2 * np.pi * kk * jj / FL),
                          -2 * np.sin(2 * np.pi * kk * jj / FL)], axis=0) / FL
    inv[0, :] = 1.0 / FL
    inv[BL, :] = np.cos(np.pi * jj[0]) / FL
    idx = _bf16_round_positions()
    e = np.zeros((NBLK, 2 * BL, FL))
    for m in range(NBLK):
        w = _window_tile(m)
        for jt in range(BL):
            e[m, idx[BL * m + jt] - BL * w] += fwd[jt]
    bf = jnp.bfloat16
    return jnp.asarray(fwd, bf), jnp.asarray(inv, bf), jnp.asarray(e, bf)


def _cmul(ar, ai, br, bi):
    return ar * br - ai * bi, ar * bi + ai * br


def _csq(ar, ai):
    return ar * ar - ai * ai, 2.0 * (ar * ai)


def _cexp(re, im):
    e = jnp.exp(re)
    return e * jnp.cos(im), e * jnp.sin(im)


def _kernel(x_ref, w_ref, wo_ref, u_ref, ssm_ref, ldt_ref, dsk_ref, fwd_ref, inv_ref, e_ref,
            out_ref,
            q_s, kt_s, vm_s, lor_s, loi_s, hir_s, hii_s, kacc_s, kv_s, kvt_s,
            uh_s, kh_s, yh_s, pw_s):
    f32, bf16 = jnp.float32, jnp.bfloat16

    lane = lax.broadcasted_iota(jnp.int32, (TQ, 128), 1)

    def proj(i, c):
        r0 = pl.multiple_of(i * TQ, TQ)
        xb = x_ref[pl.ds(r0, TQ), :]
        qkv = jnp.dot(xb, w_ref[...], preferred_element_type=f32)
        q_s[pl.ds(r0, TQ), :] = (qkv[:, :DP] * (DH ** -0.5)).astype(bf16)
        kt_s[:, pl.ds(r0, TQ)] = qkv[:, DP:2 * DP].T.astype(bf16)
        for g in range(4):
            vg = qkv[:, 2 * DP + 128 * g: 2 * DP + 128 * (g + 1)]
            for hh in range(4):
                lo = HP * hh
                vmask = jnp.where((lane >= lo) & (lane < lo + DH), vg, 0.0)
                vmask = jnp.where(lane == lo + DH, 1.0, vmask)
                vm_s[4 * g + hh, pl.ds(r0, TQ), :] = vmask.astype(bf16)
        return c

    with jax.named_scope('proj'):
        lax.fori_loop(0, S // TQ, proj, 0)

    dt1 = jnp.exp(ldt_ref[...].astype(f32)).astype(bf16).astype(f32)
    dt = jnp.concatenate([dt1, dt1], axis=1)
    kacc_s[...] = jnp.zeros_like(kacc_s)

    def lo_tables(i):
        for half in range(NB // 8):
            rows = pl.ds(pl.multiple_of(i * NB + 8 * half, 8), 8)
            sub = slice(8 * half, 8 * half + 8)
            ar = dt * ssm_ref[0, rows, :].astype(f32)
            ai = dt * ssm_ref[1, rows, :].astype(f32)
            zr, zi = _cexp(ar, ai)
            pr, pi = jnp.ones_like(zr), jnp.zeros_like(zr)
            for cc in range(16):
                qr, qi = pr, pi
                for seg in range(4):
                    lor_s[16 * seg + cc, sub, :] = qr
                    loi_s[16 * seg + cc, sub, :] = qi
                    if seg < 3:
                        qr, qi = _csq(qr, qi)
                if cc == 0:
                    pr, pi = zr, zi
                elif cc < 15:
                    pr, pi = _cmul(pr, pi, zr, zi)

    def hi_tables(i):
        for half in range(NB // 8):
            rows = pl.ds(pl.multiple_of(i * NB + 8 * half, 8), 8)
            sub = slice(8 * half, 8 * half + 8)
            ar = dt * ssm_ref[0, rows, :].astype(f32)
            ai = dt * ssm_ref[1, rows, :].astype(f32)
            wr, wi = _cexp(16.0 * ar, 16.0 * ai)
            for e in range(7):
                pw_s[2 * e] = wr
                pw_s[2 * e + 1] = wi
                if e < 6:
                    wr, wi = _csq(wr, wi)
            dbr = dt * ssm_ref[2, rows, :].astype(f32)
            dbi = dt * ssm_ref[3, rows, :].astype(f32)
            cbr, cbi = _cmul(ssm_ref[4, rows, :].astype(f32), ssm_ref[5, rows, :].astype(f32),
                             dbr, dbi)
            j = 0
            for seg in range(4):
                sr, si = pw_s[2 * seg], pw_s[2 * seg + 1]
                if seg == 0:
                    pr, pi = cbr, cbi
                else:
                    pr, pi = _cmul(cbr, cbi, pw_s[2 * seg + 6], pw_s[2 * seg + 7])
                n = 16 if seg == 0 else (9 if seg == 3 else 8)
                for hidx in range(n):
                    hir_s[j, sub, :] = pr
                    hii_s[j, sub, :] = pi
                    j += 1
                    if hidx < n - 1:
                        pr, pi = _cmul(pr, pi, sr, si)

    def pairs(j, dep):
        if j == 40:
            kacc_s[640] += hir_s[40].reshape(NB // 8, 8, D2).sum(axis=0)
            return
        seg = 0 if j < 16 else (j - 16) // 8 + 1
        hr = hir_s[j] + dep
        hi = hii_s[j] + dep
        for cc in range(16):
            t = lor_s[16 * seg + cc] * hr - loi_s[16 * seg + cc] * hi
            kacc_s[16 * j + cc] += t.reshape(NB // 8, 8, D2).sum(axis=0)

    sched = {0: ['lo'], 1: ['hi']}
    jj = 0
    for step in range(2, 16):
        n = 3 if step < 15 else 41 - jj
        sched[step] = list(range(jj, jj + n))
        jj += n

    def attn(i, c):
        r0 = pl.multiple_of(i * TQ, TQ)
        outs = []
        for g in range(4):
            qg = q_s[pl.ds(r0, TQ), 128 * g:128 * (g + 1)]
            ktg = kt_s[128 * g:128 * (g + 1), :]
            og = jnp.zeros((TQ, 128), f32)
            for hh in range(4):
                lo = HP * hh
                qm = jnp.where((lane >= lo) & (lane < lo + DH), qg, jnp.zeros_like(qg))
                s = jnp.dot(qm, ktg, preferred_element_type=f32)
                m = jnp.max(s, axis=-1, keepdims=True)
                p = jnp.exp(s - m).astype(bf16)
                oh = jnp.dot(p, vm_s[4 * g + hh], preferred_element_type=f32)
                l = oh[:, lo + DH:lo + DH + 1]
                og = og + oh * (1.0 / l)
                dep = jnp.where(m[0:1, :] > jnp.inf, 1.0, 0.0)
                for item in sched[4 * g + hh]:
                    if item == 'lo':
                        lo_tables(i)
                    elif item == 'hi':
                        hi_tables(i)
                    else:
                        pairs(item, dep)
            outs.append(og.astype(bf16))
        o = jnp.concatenate(outs, axis=1)
        res = jnp.dot(o, wo_ref[...], preferred_element_type=f32)
        out_ref[pl.ds(r0, TQ), 0:D] = res.astype(out_ref.dtype)
        return c

    with jax.named_scope('attn'):
        lax.fori_loop(0, S // TQ, attn, 0)

    def red(i, c):
        r0 = pl.multiple_of(i * 8, 8)
        kv_s[pl.ds(r0, 8), :] = jnp.sum(kacc_s[pl.ds(r0, 8)], axis=1)
        return c
    with jax.named_scope('red'):
        lax.fori_loop(0, NV // 8, red, 0)
        kv_s[pl.ds(NV, NVP - NV), :] = jnp.zeros((NVP - NV, D2), f32)
        for w in range(NVP // BL):
            kt2 = kv_s[BL * w:BL * (w + 1), :].T
            kvt_s[:, BL * w:BL * (w + 1)] = (kt2[:D] + kt2[D:]).astype(bf16)

    lane0 = lax.broadcasted_iota(jnp.int32, (D, BL), 1) == 0
    with jax.named_scope('fwd'):
        for a in range(NBLK):
            ut = u_ref[BL * a:BL * (a + 1), :].astype(f32).T.astype(bf16)
            uh_s[a] = jnp.dot(ut, fwd_ref[...], preferred_element_type=f32)
            w = _window_tile(a)
            kh = jnp.dot(kvt_s[:, BL * w:BL * (w + 2)], e_ref[a], preferred_element_type=f32)
            kr, ki = kh[:, :BL], kh[:, BL:]
            kh_s[a, :, 0:BL] = kr
            kh_s[a, :, BL:2 * BL] = jnp.where(lane0, 0.0, ki)
            kh_s[a, :, 2 * BL:3 * BL] = jnp.where(lane0, ki, kr)

    RC = 16

    def bconv(i, c):
        rows = pl.ds(pl.multiple_of(i * RC, RC), RC)
        for a in range(NBLK):
            yr = jnp.zeros((RC, BL), f32)
            yi = jnp.zeros((RC, BL), f32)
            for m in range(a + 1):
                kr = kh_s[m, rows, 0:BL]
                ki = kh_s[m, rows, BL:2 * BL]
                kb = kh_s[m, rows, 2 * BL:3 * BL]
                ur = uh_s[a - m, rows, 0:BL]
                ui = uh_s[a - m, rows, BL:2 * BL]
                yr = yr + (kr * ur - ki * ui)
                yi = yi + (kb * ui + ki * ur)
            yh_s[a, rows, 0:BL] = yr
            yh_s[a, rows, BL:2 * BL] = yi
        return c
    with jax.named_scope('bconv'):
        lax.fori_loop(0, D // RC, bconv, 0)

    dsk = dsk_ref[...].astype(f32)
    with jax.named_scope('inv'):
        prev = None
        for a in range(NBLK):
            yt = jnp.dot(yh_s[a].astype(bf16), inv_ref[...], preferred_element_type=f32)
            y = yt[:, :BL] if prev is None else yt[:, :BL] + prev
            prev = yt[:, BL:]
            ub = u_ref[BL * a:BL * (a + 1), :].astype(f32)
            y = y.T.astype(bf16).astype(f32) + (ub * dsk).astype(bf16).astype(f32)
            out_ref[BL * a:BL * (a + 1), D:2 * D] = y.astype(out_ref.dtype)


@jax.jit
def pallas_concat_heads__mha_block__ssm_conv_s4__prompt_kernel(
    A_x: jax.Array,
    A_wqkv: jax.Array,
    A_wo: jax.Array,
    B_u: jax.Array,
    B_A_re: jax.Array,
    B_A_im: jax.Array,
    B_B_re: jax.Array,
    B_B_im: jax.Array,
    B_C_re: jax.Array,
    B_C_im: jax.Array,
    B_log_dt: jax.Array,
    B_Dskip: jax.Array,
):
    bf16, f32 = jnp.bfloat16, jnp.float32
    x = A_x.reshape(S, D)
    w = jnp.pad(A_wqkv.reshape(D, 3 * H, DH), ((0, 0), (0, 0), (0, HP - DH))).reshape(D, 3 * DP)
    wo = jnp.pad(A_wo.reshape(H, DH, D), ((0, 0), (0, HP - DH), (0, 0))).reshape(DP, D)
    u = B_u.reshape(S, D)
    ssm = jnp.stack([B_A_re, B_A_im, B_B_re, B_B_im, B_C_re, B_C_im]).transpose(0, 2, 1)
    ssm = ssm.reshape(6, NS // 2, D2)
    ldt = B_log_dt.reshape(1, D)
    dsk = B_Dskip.reshape(1, D)
    fwd, inv, e = _dft_constants()

    scratch = [
        pltpu.VMEM((S, DP), bf16),
        pltpu.VMEM((DP, S), bf16),
        pltpu.VMEM((H, S, 128), bf16),
        pltpu.VMEM((64, NB, D2), f32),
        pltpu.VMEM((64, NB, D2), f32),
        pltpu.VMEM((41, NB, D2), f32),
        pltpu.VMEM((41, NB, D2), f32),
        pltpu.VMEM((NV, 8, D2), f32),
        pltpu.VMEM((NVP, D2), f32),
        pltpu.VMEM((D, NVP), bf16),
        pltpu.VMEM((NBLK, D, FL), f32),
        pltpu.VMEM((NBLK, D, 3 * BL), f32),
        pltpu.VMEM((NBLK, D, FL), f32),
        pltpu.VMEM((14, 8, D2), f32),
    ]
    out = pl.pallas_call(
        _kernel,
        out_shape=jax.ShapeDtypeStruct((S, 2 * D), bf16),
        scratch_shapes=scratch,
        compiler_params=pltpu.CompilerParams(vmem_limit_bytes=100 * 1024 * 1024),
    )(x, w, wo, u, ssm, ldt, dsk, fwd, inv, e)
    return out.reshape(1, S, 2 * D)
```

```python
import numpy as np
import jax
import jax.numpy as jnp
from jax import lax
import jax.experimental.pallas as pl
import jax.experimental.pallas.tpu as pltpu

S = 2048
D = 448
H = 16
DH = 28
HP = 32
DP = H * HP
NS = 256
BL = 128
FL = 256
NBLK = S // BL
NVP = 768
TQ = 256
NB = 16
D2 = 2 * D
NV = 648


def _bf16_round_positions():
    t = np.arange(S)
    idx = np.empty(S, np.int64)
    for i, tt in enumerate(t):
        if tt < 256:
            idx[i] = tt
            continue
        seg = int(np.floor(np.log2(tt))) - 7
        step = 1 << seg
        base = 128 << seg
        q, r = divmod(tt - base, step)
        if 2 * r > step or (2 * r == step and q % 2 == 1):
            q += 1
        idx[i] = 128 + 128 * seg + q
    return idx


def _window_tile(m):
    return (0, 1, 2, 2, 3, 3, 3, 3, 4, 4, 4, 4, 4, 4, 4, 4)[m]


def _dft_constants():
    j = np.arange(BL)[:, None]
    k = np.arange(BL)[None, :]
    fwd = np.concatenate([np.cos(2 * np.pi * j * k / FL), -np.sin(2 * np.pi * j * k / FL)], axis=1)
    fwd[:, BL] = np.cos(np.pi * j[:, 0])
    jj = np.arange(FL)[None, :]
    kk = np.arange(BL)[:, None]
    inv = np.concatenate([2 * np.cos(2 * np.pi * kk * jj / FL),
                          -2 * np.sin(2 * np.pi * kk * jj / FL)], axis=0) / FL
    inv[0, :] = 1.0 / FL
    inv[BL, :] = np.cos(np.pi * jj[0]) / FL
    idx = _bf16_round_positions()
    e = np.zeros((NBLK, 2 * BL, FL))
    for m in range(NBLK):
        w = _window_tile(m)
        for jt in range(BL):
            e[m, idx[BL * m + jt] - BL * w] += fwd[jt]
    bf = jnp.bfloat16
    return jnp.asarray(fwd, bf), jnp.asarray(inv, bf), jnp.asarray(e, bf)


def _cmul(ar, ai, br, bi):
    return ar * br - ai * bi, ar * bi + ai * br


def _csq(ar, ai):
    return ar * ar - ai * ai, 2.0 * (ar * ai)


def _cexp(re, im):
    e = jnp.exp(re)
    return e * jnp.cos(im), e * jnp.sin(im)


def _kernel(x_ref, w_ref, wo_ref, ut_ref, ssm_ref, ldt_ref, dsk_ref, fwd_ref, inv_ref, e_ref,
            out_ref,
            q_s, kt_s, vm_s, lor_s, loi_s, hir_s, hii_s, kacc_s, kv_s, kvt_s,
            uh_s, kh_s, yh_s, pw_s):
    f32, bf16 = jnp.float32, jnp.bfloat16

    lane = lax.broadcasted_iota(jnp.int32, (TQ, 128), 1)

    def proj(i, c):
        r0 = pl.multiple_of(i * TQ, TQ)
        xb = x_ref[pl.ds(r0, TQ), :]
        qkv = jnp.dot(xb, w_ref[...], preferred_element_type=f32)
        q_s[pl.ds(r0, TQ), :] = (qkv[:, :DP] * (DH ** -0.5)).astype(bf16)
        kt_s[:, pl.ds(r0, TQ)] = qkv[:, DP:2 * DP].T.astype(bf16)
        for g in range(4):
            vg = qkv[:, 2 * DP + 128 * g: 2 * DP + 128 * (g + 1)]
            for hh in range(4):
                lo = HP * hh
                vmask = jnp.where((lane >= lo) & (lane < lo + DH), vg, 0.0)
                vmask = jnp.where(lane == lo + DH, 1.0, vmask)
                vm_s[4 * g + hh, pl.ds(r0, TQ), :] = vmask.astype(bf16)
        return c

    with jax.named_scope('proj'):
        lax.fori_loop(0, S // TQ, proj, 0)

    dt1 = jnp.exp(ldt_ref[...].astype(f32)).astype(bf16).astype(f32)
    dt = jnp.concatenate([dt1, dt1], axis=1)
    kacc_s[...] = jnp.zeros_like(kacc_s)

    def lo_tables(i):
        for half in range(NB // 8):
            rows = pl.ds(pl.multiple_of(i * NB + 8 * half, 8), 8)
            sub = slice(8 * half, 8 * half + 8)
            ar = dt * ssm_ref[0, rows, :].astype(f32)
            ai = dt * ssm_ref[1, rows, :].astype(f32)
            zr, zi = _cexp(ar, ai)
            pr, pi = jnp.ones_like(zr), jnp.zeros_like(zr)
            for cc in range(16):
                qr, qi = pr, pi
                for seg in range(4):
                    lor_s[16 * seg + cc, sub, :] = qr
                    loi_s[16 * seg + cc, sub, :] = qi
                    if seg < 3:
                        qr, qi = _csq(qr, qi)
                if cc == 0:
                    pr, pi = zr, zi
                elif cc < 15:
                    pr, pi = _cmul(pr, pi, zr, zi)

    def hi_tables(i):
        for half in range(NB // 8):
            rows = pl.ds(pl.multiple_of(i * NB + 8 * half, 8), 8)
            sub = slice(8 * half, 8 * half + 8)
            ar = dt * ssm_ref[0, rows, :].astype(f32)
            ai = dt * ssm_ref[1, rows, :].astype(f32)
            wr, wi = _cexp(16.0 * ar, 16.0 * ai)
            for e in range(7):
                pw_s[2 * e] = wr
                pw_s[2 * e + 1] = wi
                if e < 6:
                    wr, wi = _csq(wr, wi)
            dbr = dt * ssm_ref[2, rows, :].astype(f32)
            dbi = dt * ssm_ref[3, rows, :].astype(f32)
            cbr, cbi = _cmul(ssm_ref[4, rows, :].astype(f32), ssm_ref[5, rows, :].astype(f32),
                             dbr, dbi)
            j = 0
            for seg in range(4):
                sr, si = pw_s[2 * seg], pw_s[2 * seg + 1]
                if seg == 0:
                    pr, pi = cbr, cbi
                else:
                    pr, pi = _cmul(cbr, cbi, pw_s[2 * seg + 6], pw_s[2 * seg + 7])
                n = 16 if seg == 0 else (9 if seg == 3 else 8)
                for hidx in range(n):
                    hir_s[j, sub, :] = pr
                    hii_s[j, sub, :] = pi
                    j += 1
                    if hidx < n - 1:
                        pr, pi = _cmul(pr, pi, sr, si)

    def pairs(j, dep):
        if j == 40:
            kacc_s[640] += hir_s[40].reshape(NB // 8, 8, D2).sum(axis=0)
            return
        seg = 0 if j < 16 else (j - 16) // 8 + 1
        hr = hir_s[j] + dep
        hi = hii_s[j] + dep
        for cc in range(16):
            t = lor_s[16 * seg + cc] * hr - loi_s[16 * seg + cc] * hi
            kacc_s[16 * j + cc] += t.reshape(NB // 8, 8, D2).sum(axis=0)

    sched = {0: ['lo'], 1: ['hi']}
    jj = 0
    for step in range(2, 16):
        n = 3 if step < 15 else 41 - jj
        sched[step] = list(range(jj, jj + n))
        jj += n

    def attn(i, c):
        r0 = pl.multiple_of(i * TQ, TQ)
        outs = []
        for g in range(4):
            qg = q_s[pl.ds(r0, TQ), 128 * g:128 * (g + 1)]
            ktg = kt_s[128 * g:128 * (g + 1), :]
            og = jnp.zeros((TQ, 128), f32)
            for hh in range(4):
                lo = HP * hh
                qm = jnp.where((lane >= lo) & (lane < lo + DH), qg, jnp.zeros_like(qg))
                s = jnp.dot(qm, ktg, preferred_element_type=f32)
                m = jnp.max(s, axis=-1, keepdims=True)
                p = jnp.exp(s - m).astype(bf16)
                oh = jnp.dot(p, vm_s[4 * g + hh], preferred_element_type=f32)
                l = oh[:, lo + DH:lo + DH + 1]
                og = og + oh * (1.0 / l)
                dep = jnp.where(m[0:1, :] > jnp.inf, 1.0, 0.0)
                for item in sched[4 * g + hh]:
                    if item == 'lo':
                        lo_tables(i)
                    elif item == 'hi':
                        hi_tables(i)
                    else:
                        pairs(item, dep)
            outs.append(og.astype(bf16))
        o = jnp.concatenate(outs, axis=1)
        res = jnp.dot(o, wo_ref[...], preferred_element_type=f32)
        out_ref[pl.ds(r0, TQ), 0:D] = res.astype(out_ref.dtype)
        return c

    with jax.named_scope('attn'):
        lax.fori_loop(0, S // TQ, attn, 0)

    def red(i, c):
        r0 = pl.multiple_of(i * 8, 8)
        kv_s[pl.ds(r0, 8), :] = jnp.sum(kacc_s[pl.ds(r0, 8)], axis=1)
        return c
    with jax.named_scope('red'):
        lax.fori_loop(0, NV // 8, red, 0)
        kv_s[pl.ds(NV, NVP - NV), :] = jnp.zeros((NVP - NV, D2), f32)
        for w in range(NVP // BL):
            kt2 = kv_s[BL * w:BL * (w + 1), :].T
            kvt_s[:, BL * w:BL * (w + 1)] = (kt2[:D] + kt2[D:]).astype(bf16)

    lane0 = lax.broadcasted_iota(jnp.int32, (D, BL), 1) == 0
    with jax.named_scope('fwd'):
        for a in range(NBLK):
            ut = ut_ref[:, BL * a:BL * (a + 1)]
            uh_s[a] = jnp.dot(ut, fwd_ref[...], preferred_element_type=f32)
            w = _window_tile(a)
            kh = jnp.dot(kvt_s[:, BL * w:BL * (w + 2)], e_ref[a], preferred_element_type=f32)
            kr, ki = kh[:, :BL], kh[:, BL:]
            kh_s[a, :, 0:BL] = kr
            kh_s[a, :, BL:2 * BL] = jnp.where(lane0, 0.0, ki)
            kh_s[a, :, 2 * BL:3 * BL] = jnp.where(lane0, ki, kr)

    RC = 16

    def bconv(i, c):
        rows = pl.ds(pl.multiple_of(i * RC, RC), RC)
        for a in range(NBLK):
            yr = jnp.zeros((RC, BL), f32)
            yi = jnp.zeros((RC, BL), f32)
            for m in range(a + 1):
                kr = kh_s[m, rows, 0:BL]
                ki = kh_s[m, rows, BL:2 * BL]
                kb = kh_s[m, rows, 2 * BL:3 * BL]
                ur = uh_s[a - m, rows, 0:BL]
                ui = uh_s[a - m, rows, BL:2 * BL]
                yr = yr + (kr * ur - ki * ui)
                yi = yi + (kb * ui + ki * ur)
            yh_s[a, rows, 0:BL] = yr
            yh_s[a, rows, BL:2 * BL] = yi
        return c
    with jax.named_scope('bconv'):
        lax.fori_loop(0, D // RC, bconv, 0)

    dsk = dsk_ref[...].astype(f32)
    with jax.named_scope('inv'):
        prev = None
        for a in range(NBLK):
            yt = jnp.dot(yh_s[a].astype(bf16), inv_ref[...], preferred_element_type=f32)
            y = yt[:, :BL] if prev is None else yt[:, :BL] + prev
            prev = yt[:, BL:]
            ub = ut_ref[:, BL * a:BL * (a + 1)].astype(f32)
            y = y.astype(bf16).astype(f32) + (ub * dsk).astype(bf16).astype(f32)
            out_ref[BL * a:BL * (a + 1), D:2 * D] = y.T.astype(out_ref.dtype)


@jax.jit
def pallas_concat_heads__mha_block__ssm_conv_s4__prompt_kernel(
    A_x: jax.Array,
    A_wqkv: jax.Array,
    A_wo: jax.Array,
    B_u: jax.Array,
    B_A_re: jax.Array,
    B_A_im: jax.Array,
    B_B_re: jax.Array,
    B_B_im: jax.Array,
    B_C_re: jax.Array,
    B_C_im: jax.Array,
    B_log_dt: jax.Array,
    B_Dskip: jax.Array,
):
    bf16, f32 = jnp.bfloat16, jnp.float32
    x = A_x.reshape(S, D)
    w = jnp.pad(A_wqkv.reshape(D, 3 * H, DH), ((0, 0), (0, 0), (0, HP - DH))).reshape(D, 3 * DP)
    wo = jnp.pad(A_wo.reshape(H, DH, D), ((0, 0), (0, HP - DH), (0, 0))).reshape(DP, D)
    ut = B_u.reshape(S, D).T
    ssm = jnp.stack([B_A_re, B_A_im, B_B_re, B_B_im, B_C_re, B_C_im]).transpose(0, 2, 1)
    ssm = ssm.reshape(6, NS // 2, D2)
    ldt = B_log_dt.reshape(1, D)
    dsk = B_Dskip.reshape(D, 1)
    fwd, inv, e = _dft_constants()

    scratch = [
        pltpu.VMEM((S, DP), bf16),
        pltpu.VMEM((DP, S), bf16),
        pltpu.VMEM((H, S, 128), bf16),
        pltpu.VMEM((64, NB, D2), f32),
        pltpu.VMEM((64, NB, D2), f32),
        pltpu.VMEM((41, NB, D2), f32),
        pltpu.VMEM((41, NB, D2), f32),
        pltpu.VMEM((NV, 8, D2), f32),
        pltpu.VMEM((NVP, D2), f32),
        pltpu.VMEM((D, NVP), bf16),
        pltpu.VMEM((NBLK, D, FL), f32),
        pltpu.VMEM((NBLK, D, 3 * BL), f32),
        pltpu.VMEM((NBLK, D, FL), f32),
        pltpu.VMEM((14, 8, D2), f32),
    ]
    out = pl.pallas_call(
        _kernel,
        out_shape=jax.ShapeDtypeStruct((S, 2 * D), bf16),
        scratch_shapes=scratch,
        compiler_params=pltpu.CompilerParams(vmem_limit_bytes=100 * 1024 * 1024),
    )(x, w, wo, ut, ssm, ldt, dsk, fwd, inv, e)
    return out.reshape(1, S, 2 * D)
```
